```python
import os as _os
_os.environ.setdefault("JAX_PLATFORMS", "cpu")
import jax
import jax.numpy as jnp

def _softmax(x, axis=-1):
    return jax.nn.softmax(x, axis=axis)
def _gelu(x):
    return jax.nn.gelu(x, approximate=True)
def _silu(x):
    return jax.nn.silu(x)
def _sigmoid(x):
    return jax.nn.sigmoid(x)
def _layernorm(x, axis=-1, eps=1e-5):
    m = jnp.mean(x, axis=axis, keepdims=True)
    v = jnp.var(x, axis=axis, keepdims=True)
    return (x - m) / jnp.sqrt(v + eps)
def _scatter_add(tgt, idx, src, axis=0):
    return tgt.at[idx].add(src)
def _segment_sum(src, seg, n):
    return jax.ops.segment_sum(src, seg, n)
class _Rng:
    def __init__(self, key):
        self._k = key
    def _next(self):
        self._k, sub = jax.random.split(self._k)
        return sub
    def normal(self, shape):
        return jax.random.normal(self._next(), shape, dtype=jnp.bfloat16)
    def randint(self, lo, hi, shape):
        return jax.random.randint(self._next(), shape, lo, hi, dtype=jnp.int32)
    def uniform(self, shape, lo=0.0, hi=1.0):
        return jax.random.uniform(self._next(), shape, jnp.bfloat16, lo, hi)
    def permutation(self, n):
        return jax.random.permutation(self._next(), n)


kernel_name = 'parallel_sum__sliding_block__moe_arch_mod__prompt'

def setup_inputs():
    _rng = _Rng(jax.random.key(int.from_bytes(__import__("os").urandom(4), "little")))
    _w = (lambda a: (lambda t: t.astype(jnp.bfloat16) if jnp.issubdtype(t.dtype, jnp.floating) else t)(jnp.asarray(a)))
    def _A_setup():
        B, S, D = 1, 2048, 512
        return {
            "x": _w((lambda *s: _rng.normal(s) * 0.05)(B, S, D)),
            "wqkv": _w((lambda *s: _rng.normal(s) * 0.05)(D, 3 * D)),
            "wo": _w((lambda *s: _rng.normal(s) * 0.05)(D, D)),
        }
    _A_in = _A_setup()

    def _B_setup():
        B, S, D, F, C = 1, 2048, 512, 1376, 1
        return {
            "x": _w((lambda *s: _rng.normal(s) * 0.05)(B, S, D)),
            "w_r": _w((lambda *s: _rng.normal(s) * 0.05)(D)),
            "w_gate": _w((lambda *s: _rng.normal(s) * 0.05)(D, F)),
            "w_up": _w((lambda *s: _rng.normal(s) * 0.05)(D, F)),
            "w_down": _w((lambda *s: _rng.normal(s) * 0.05)(F, D)),
        }
    _B_in = _B_setup()

    return {
        "A_x": _A_in["x"],
        "A_wqkv": _A_in["wqkv"],
        "A_wo": _A_in["wo"],
        "B_x": _B_in["x"],
        "B_w_r": _B_in["w_r"],
        "B_w_gate": _B_in["w_gate"],
        "B_w_up": _B_in["w_up"],
        "B_w_down": _B_in["w_down"],
    }

def reference(A_x, A_wqkv, A_wo, B_x, B_w_r, B_w_gate, B_w_up, B_w_down):
    def _A_ref(x, wqkv, wo):
        B, S, D = x.shape
        H = 32; Dh = D // H; W = 256
        qkv = (lambda x, *d: x.transpose(*d))((x @ wqkv).reshape(B, S, 3, H, Dh), 2, 0, 3, 1, 4)
        q, k, v = qkv[0], qkv[1], qkv[2]
        scores = jnp.einsum("bhqd,bhkd->bhqk", q, k) * (Dh ** -0.5)
        idx = jnp.arange(S)
        mask = (idx[:, None] - idx[None, :] >= 0) & (idx[:, None] - idx[None, :] < W)
        scores = jnp.where(mask[None, None], scores, -1e9)
        p = _softmax(scores, axis=-1)
        o = jnp.einsum("bhqk,bhkd->bhqd", p, v)
        return (lambda x, *d: x.transpose(*d))(o, 0, 2, 1, 3).reshape(B, S, D) @ wo

    def _B_ref(x, w_r, w_gate, w_up, w_down):
        B, S, D = x.shape
        C = 1
        r = x @ w_r
        idx = jnp.argsort(-r, axis=-1)[:, :C]
        idx_e = jnp.repeat(idx.reshape(B, C, 1), D, axis=2)
        x_sel = jnp.take_along_axis(x, idx_e, axis=1)
        g = _silu(x_sel @ w_gate)
        u = x_sel @ w_up
        y = (g * u) @ w_down
        r_sel = _sigmoid(jnp.take_along_axis(r, idx, axis=1))
        y = y * r_sel.reshape(B, C, 1)
        b_off = (jnp.arange(B) * S).reshape(B, 1)
        flat_idx = (idx + b_off).reshape(B * C)
        zero = (x * 0.0).reshape(B * S, D)
        upd = _scatter_add(zero, flat_idx, y.reshape(B * C, D), axis=0)
        return x + upd.reshape(B, S, D)

    x = A_x
    xn = _layernorm(x, axis=-1)
    return x + _A_ref(xn, A_wqkv, A_wo) + _B_ref(xn, B_w_r, B_w_gate, B_w_up, B_w_down)
```

```python
import jax
import jax.numpy as jnp
from jax import lax
import jax.experimental.pallas as pl
import jax.experimental.pallas.tpu as pltpu

S, D, H, DH, W, F = 2048, 512, 32, 16, 256, 1376
QB = 128
NQ = S // QB
LOG2E = 1.4426950408889634
QSCALE = (DH ** -0.5) * LOG2E
NEG = -1e30
FMAX = 3.0e38
L_LO, L_HI = 2.0 ** -60, 2.0 ** 60
RB = 512
KB = 256
LNC = 16
XD = (256, 256, 512, 1024)
XO = (0, 256, 512, 1024)
PEEL, UNR = 2, 2
NACC = 8

NT = (((1,), (1,)), ((), ()))
TN = (((0,), (0,)), ((), ()))
f32, bf16, u32 = jnp.float32, jnp.bfloat16, jnp.uint32


def _pk(x):
    return pltpu.bitcast(x, u32)


def _upk(x):
    return pltpu.bitcast(x, bf16)


def _kernel(x_hbm, wqkv_hbm, wo_hbm, wr_hbm, wg_hbm, wu_hbm, wd_hbm, o_hbm,
            x_v, wqkv_v, wo_v, wr_v, wg_v, wu_v, wd_v,
            wt_v, wo_p, xn_v, k_v, qm_v, vt_v, wrb_v, y_v, ot_v, out_v, b0_v, b4_v, p_s, l_s, z_s,
            sem_x, sem_w, sem_o):
    def xcopy(i):
        return pltpu.make_async_copy(x_hbm.at[pl.ds(XO[i], XD[i]), :], x_v.at[pl.ds(XO[i], XD[i]), :], sem_x.at[i])

    def wcopy(j):
        return pltpu.make_async_copy(wqkv_hbm.at[:, pl.ds(j * D, D)], wqkv_v.at[:, pl.ds(j * D, D)], sem_w.at[j])

    cp = {
        'wq': wcopy(0), 'wk': wcopy(1), 'wv': wcopy(2),
        'wr': pltpu.make_async_copy(wr_hbm, wr_v, sem_w.at[3]),
        'wo': pltpu.make_async_copy(wo_hbm, wo_v, sem_w.at[4]),
        'wg': pltpu.make_async_copy(wg_hbm, wg_v, sem_w.at[5]),
        'wu': pltpu.make_async_copy(wu_hbm, wu_v, sem_w.at[6]),
        'wd': pltpu.make_async_copy(wd_hbm, wd_v, sem_w.at[7]),
    }
    for i in range(len(XD)):
        cp[f'x{i}'] = xcopy(i)
    plan = {'start': ('x0', 'wr', 'wk'), 'x0': ('x1', 'x2'), 'x1': ('x3',), 'x2': ('wq', 'wv'),
            'x3': ('wg', 'wu', 'wd', 'wo')}

    def fire(point):
        for name in plan[point]:
            cp[name].start()

    x_waited = set()

    def need_rows(r1):
        for j in range(len(XD)):
            if XO[j] < r1 and j not in x_waited:
                x_waited.add(j)
                cp[f'x{j}'].wait()
                fire(f'x{j}')

    fire('start')

    ri = lax.broadcasted_iota(jnp.int32, (64, 128), 0)
    ci = lax.broadcasted_iota(jnp.int32, (64, 128), 1) & 63
    b0_v[...] = jnp.where(ri > ci, 0.0, NEG).astype(f32)
    b4_v[...] = jnp.where(ri <= ci, 0.0, NEG).astype(f32)
    for p in range(4):
        p_s[0, p, 160:192, :] = jnp.zeros((32, 128), u32)
        p_s[1, p, 0:32, :] = jnp.zeros((32, 128), u32)
    y_v[...] = jnp.zeros(y_v.shape, f32)
    lo = lax.broadcasted_iota(jnp.int32, (8, 128), 1) < 64

    def layer_norm(xb):
        mean = jnp.mean(xb, axis=-1, keepdims=True)
        xc = xb - mean
        var = jnp.mean(xc * xc, axis=-1, keepdims=True)
        return xc * lax.rsqrt(var + 1e-5)

    router = {}
    row16 = lax.broadcasted_iota(jnp.int32, (LNC, 1), 0)

    def ln_block(i):
        for c in range(KB // LNC):
            r0 = i * KB + c * LNC
            xnf = layer_norm(x_v[r0:r0 + LNC, :].astype(f32))
            xn_v[r0:r0 + LNC, :] = xnf.astype(bf16)
            rr = jnp.sum(xnf * wrb_v[0:1, :], axis=1, keepdims=True).astype(bf16).astype(f32)
            if 'best' not in router:
                router['best'], router['idx'] = rr, row16 + r0
            else:
                better = rr > router['best']
                router['best'] = jnp.where(better, rr, router['best'])
                router['idx'] = jnp.where(better, row16 + r0, router['idx'])

    def k_block(i):
        xn = xn_v[i * KB:(i + 1) * KB, :]
        kk = jnp.dot(xn, wqkv_v[:, D:2 * D], preferred_element_type=f32)
        k_v[pl.ds(i * KB // 2, KB // 2), :] = _pk(kk.astype(bf16))

    def qv_block(i):
        xn = xn_v[i * RB:(i + 1) * RB, :]
        qv = lax.dot_general(_upk(wt_v[...]), xn, NT, preferred_element_type=f32)
        for j in range(RB // 128):
            a = i * (RB // 128) + j
            cols = slice(j * 128, (j + 1) * 128)
            vt_v[a] = _pk(qv[D:2 * D, cols].astype(bf16))
            qp = _pk((qv[0:D, cols] * QSCALE).astype(bf16))
            for h in range(H):
                q = qp[8 * h:8 * h + 8]
                if h % 2 == 0:
                    qm_v[a, 0, 8 * h:8 * h + 8] = jnp.where(lo, q, 0)
                    qm_v[a, 1, 8 * h:8 * h + 8] = jnp.where(lo, 0, q)
                else:
                    r = pltpu.roll(q, 64, 1)
                    qm_v[a, 0, 8 * h:8 * h + 8] = jnp.where(lo, 0, r)
                    qm_v[a, 1, 8 * h:8 * h + 8] = jnp.where(lo, r, 0)

    nkb = S // KB
    cp['wr'].wait()
    need_rows(KB)
    wr4 = wr_v[...].astype(f32).reshape(4, 128)
    wrb_v[...] = jnp.broadcast_to(jnp.concatenate([wr4[j:j + 1, :] for j in range(4)], axis=1), (8, D))
    ln_block(0)
    cp['wk'].wait()
    for i in range(nkb):
        if i + 1 < nkb:
            need_rows((i + 2) * KB)
        if i == nkb - 1:
            cp['wq'].wait()
            cp['wv'].wait()
        k_block(i)
        if i + 1 < nkb:
            ln_block(i + 1)
        if i == nkb - 1:
            wt_v[0:D // 2, :] = _pk(wqkv_v[:, 0:D].T)
            wt_v[D // 2:D, :] = _pk(wqkv_v[:, 2 * D:3 * D].T)

    rmax = jnp.max(router['best'])
    idx = jnp.min(jnp.where(router['best'] == rmax, router['idx'], S))
    idx = jnp.minimum(idx, S - 1)
    base = pl.multiple_of((idx // 16) * 16, 16)
    rsel = lax.broadcasted_iota(jnp.int32, (16, D), 0) == (idx - base)

    def ffn():
        xs = xn_v[pl.ds(base, 16), :].astype(f32)
        xb = jnp.broadcast_to(jnp.sum(jnp.where(rsel, xs, 0.0), axis=0, keepdims=True), (16, D))
        nc = F // 16
        accs = [None] * NACC
        for c in range(nc):
            f0 = 16 * c
            g = jnp.sum(wg_v[f0:f0 + 16, :].astype(f32) * xb, axis=1, keepdims=True)
            u = jnp.sum(wu_v[f0:f0 + 16, :].astype(f32) * xb, axis=1, keepdims=True)
            hh = (g * jax.nn.sigmoid(g) * u).astype(bf16).astype(f32)
            t = hh * wd_v[f0:f0 + 16, :].astype(f32)
            j = c * NACC // nc
            accs[j] = t if accs[j] is None else accs[j] + t
        acc = accs[0]
        for extra in accs[1:]:
            acc = acc + extra
        y = jnp.sum(acc, axis=0, keepdims=True) * jax.nn.sigmoid(jnp.full((1, D), rmax, f32))
        y_v[pl.ds(pl.multiple_of(base % QB, 16) + QB, 16), :] = jnp.where(rsel, y, 0.0)

    for i in range(S // RB):
        if i == 2:
            for name in ('wg', 'wu', 'wd'):
                cp[name].wait()
        qv_block(i)
        if i == 3:
            ffn()
    cp['wo'].wait()
    yblk = idx // QB
    wo_p[...] = _pk(wo_v[...])

    def ocopy(a):
        rows = pl.ds(pl.multiple_of(a * QB, QB), QB)
        return pltpu.make_async_copy(out_v.at[rows, :], o_hbm.at[rows, :], sem_o.at[0])

    def q_tile(a, e, g, p):
        r0 = (g * 128 + p * 32) // 2
        parts = []
        if p > 0:
            parts.append(jnp.zeros((32 * p, 128), bf16))
        parts.append(_upk(qm_v[a, e, r0:r0 + 16, :]))
        if p < 3:
            parts.append(jnp.zeros((32 * (3 - p), 128), bf16))
        return jnp.concatenate(parts, axis=0)

    chk = [jnp.ones((1, 128), f32), jnp.ones((1, 128), f32), jnp.zeros((8, 128), f32)]

    def stage_a(a, e, g, c0):
        if isinstance(a, int):
            kstart = (2 * a + e - 4 + c0) * 32
        else:
            kstart = pl.multiple_of((2 * a + e - 4) * 32, 32)
        kwin = _upk(k_v[pl.ds(kstart, 32 * (5 - c0)), g * 128:(g + 1) * 128])
        rhs = jnp.concatenate([q_tile(a, e, g, p) for p in range(4)], axis=1)
        st4 = jnp.dot(kwin, rhs, preferred_element_type=f32)
        for p in range(4):
            st = st4[:, p * 128:(p + 1) * 128]
            tot = None
            for c in range(c0, 5):
                sc = st[64 * (c - c0):64 * (c - c0) + 64]
                if c == 0:
                    sc = sc + b0_v[...]
                if c == 4:
                    sc = sc + b4_v[...]
                pc = jnp.exp2(sc)
                tot = pc if tot is None else tot + pc
                p_s[e, p, 32 * (c + e):32 * (c + e) + 32, :] = _pk(pc.astype(bf16))
            l = jnp.sum(tot, axis=0, keepdims=True)
            l_s[e, p] = jnp.broadcast_to(1.0 / l, (8, 128))
            chk[0] = jnp.minimum(chk[0], l)
            chk[1] = jnp.maximum(chk[1], l)

    def stage_b(a, e, g, par, t0):
        for p in range(4):
            r0 = (g * 128 + p * 32) // 2
            ot = None
            for t in range(t0, 3):
                vt = _upk(vt_v[a - 2 + t, r0:r0 + 16, :])
                r = jnp.dot(vt, _upk(p_s[e, p, 64 * t:64 * (t + 1), :]), preferred_element_type=f32)
                ot = r if ot is None else ot + r
            on = ot * jnp.concatenate([l_s[e, p]] * 4, axis=0)
            fin = jnp.abs(on) <= FMAX
            chk[2] = jnp.where(fin[0:8] & fin[8:16] & fin[16:24] & fin[24:32], chk[2], 1.0)
            z = _pk(on.astype(bf16))
            if e == 0:
                z_s[p] = z
            else:
                z0 = z_s[p]
                ot_v[par, r0:r0 + 8, :] = jnp.where(lo, z0[0:8], z[0:8])
                ot_v[par, r0 + 8:r0 + 16, :] = pltpu.roll(jnp.where(lo, z[8:16], z0[8:16]), 64, 1)

    def out_proj(a, par):
        q0 = pl.multiple_of(a * QB, QB)
        att = lax.dot_general(_upk(ot_v[par]), _upk(wo_p[...]), TN, preferred_element_type=f32)
        yoff = pl.multiple_of(jnp.where(yblk == a, QB, 0), QB)
        res = att + (x_v[pl.ds(q0, QB), :].astype(f32) + xn_v[pl.ds(q0, QB), :].astype(f32)
                     + y_v[pl.ds(yoff, QB), :])
        out_v[pl.ds(q0, QB), :] = res.astype(bf16)

    def c0_of(a, e):
        return max(0, 4 - (2 * a + e))

    def q_block(a, par, a_next, c0_next, do_out):
        static = isinstance(a, int)
        for gi in range(8):
            g, e = gi // 2, gi % 2
            if gi < 7:
                e1 = (gi + 1) % 2
                stage_a(a, e1, (gi + 1) // 2, c0_of(a, e1) if static else 0)
            else:
                stage_a(a_next, 0, 0, c0_next)
            stage_b(a, e, g, par, max(0, 2 - a) if static else 0)
        if do_out:
            out_proj(a - 1, 1 - par)

    stage_a(0, 0, 0, 4)
    for a in range(PEEL):
        q_block(a, a % 2, a + 1, c0_of(a + 1, 0), a >= 1)
        if a >= 1:
            ocopy(a - 1).start()

    def main_loop(it, carry):
        chk[:] = carry
        a0 = PEEL + it * UNR
        for u in range(UNR):
            a = a0 + u
            q_block(a, u % 2, jnp.minimum(a + 1, NQ - 1), 0, True)
            ocopy(a - 1).start()
        return tuple(chk)

    chk[:] = lax.fori_loop(0, (NQ - PEEL) // UNR, main_loop, tuple(chk))
    out_proj(NQ - 1, (NQ - 1) % 2)
    ocopy(NQ - 1).start()
    for a in range(NQ):
        ocopy(a).wait()

    ok = (chk[0] >= L_LO) & (chk[1] <= L_HI)
    nbad = jnp.sum(jnp.where(ok, 0.0, 1.0)) + jnp.sum(chk[2])

    @pl.when(nbad != 0.0)
    def _():
        row = lax.broadcasted_iota(jnp.int32, (384, 128), 0)
        col = lax.broadcasted_iota(jnp.int32, (384, 128), 1) & 63

        def safe_block(a, carry):
            tiles = [jnp.maximum(a - 2 + t, 0) for t in range(3)]
            for g in range(4):
                kwin = jnp.concatenate(
                    [_upk(k_v[pl.ds(pl.multiple_of(tl * 64, 64), 64), g * 128:(g + 1) * 128]) for tl in tiles],
                    axis=0)
                zs = [None] * 4
                for e in range(2):
                    d = 256 + 64 * e + col - row
                    valid = (d >= 0) & (d < W) & (row + 128 * (a - 2) >= 0)
                    for p in range(4):
                        r0 = (g * 128 + p * 32) // 2
                        st = jnp.dot(kwin, q_tile(a, e, g, p), preferred_element_type=f32)
                        st = jnp.where(valid, st, NEG)
                        m = jnp.max(st, axis=0, keepdims=True)
                        pe = jnp.exp2(st - m)
                        linv = 1.0 / jnp.sum(pe, axis=0, keepdims=True)
                        vt = jnp.concatenate([_upk(vt_v[tl, r0:r0 + 16, :]) for tl in tiles], axis=1)
                        ot = jnp.dot(vt, pe.astype(bf16), preferred_element_type=f32)
                        z = _pk((ot * linv).astype(bf16))
                        if e == 0:
                            zs[p] = z
                        else:
                            ot_v[0, r0:r0 + 8, :] = jnp.where(lo, zs[p][0:8], z[0:8])
                            ot_v[0, r0 + 8:r0 + 16, :] = pltpu.roll(jnp.where(lo, z[8:16], zs[p][8:16]), 64, 1)
            out_proj(a, 0)
            ocopy(a).start()
            ocopy(a).wait()
            return carry

        lax.fori_loop(0, NQ, safe_block, 0)


@jax.jit
def pallas_parallel_sum__sliding_block__moe_arch_mod__prompt_kernel(
    A_x: jax.Array,
    A_wqkv: jax.Array,
    A_wo: jax.Array,
    B_x: jax.Array,
    B_w_r: jax.Array,
    B_w_gate: jax.Array,
    B_w_up: jax.Array,
    B_w_down: jax.Array,
):
    del B_x
    hbm = pl.BlockSpec(memory_space=pltpu.HBM)
    out = pl.pallas_call(
        _kernel,
        out_shape=jax.ShapeDtypeStruct((S, D), bf16),
        in_specs=[hbm] * 7,
        out_specs=hbm,
        scratch_shapes=[
            pltpu.VMEM((S, D), bf16),
            pltpu.VMEM((D, 3 * D), bf16),
            pltpu.VMEM((D, D), bf16),
            pltpu.VMEM((D,), bf16),
            pltpu.VMEM((F, D), bf16),
            pltpu.VMEM((F, D), bf16),
            pltpu.VMEM((F, D), bf16),
            pltpu.VMEM((D, D), u32),
            pltpu.VMEM((D // 2, D), u32),
            pltpu.VMEM((S, D), bf16),
            pltpu.VMEM((S // 2, D), u32),
            pltpu.VMEM((NQ, 2, D // 2, 128), u32),
            pltpu.VMEM((NQ, D // 2, 128), u32),
            pltpu.VMEM((8, D), f32),
            pltpu.VMEM((2 * QB, D), f32),
            pltpu.VMEM((2, D // 2, 128), u32),
            pltpu.VMEM((S, D), bf16),
            pltpu.VMEM((64, 128), f32),
            pltpu.VMEM((64, 128), f32),
            pltpu.VMEM((2, 4, 192, 128), u32),
            pltpu.VMEM((2, 4, 8, 128), f32),
            pltpu.VMEM((4, 16, 128), u32),
            pltpu.SemaphoreType.DMA((len(XD),)),
            pltpu.SemaphoreType.DMA((8,)),
            pltpu.SemaphoreType.DMA((1,)),
        ],
        compiler_params=pltpu.CompilerParams(vmem_limit_bytes=80 * 2**20),
        name="fused_swa_mod",
    )(A_x.reshape(S, D), A_wqkv, A_wo, B_w_r, B_w_gate.T, B_w_up.T, B_w_down)
    return out.reshape(1, S, D)
```

```python
import jax
import jax.numpy as jnp
from jax import lax
import jax.experimental.pallas as pl
import jax.experimental.pallas.tpu as pltpu

S, D, H, DH, W, F = 2048, 512, 32, 16, 256, 1376
QB = 128
NQ = S // QB
LOG2E = 1.4426950408889634
QSCALE = (DH ** -0.5) * LOG2E
NEG = -1e30
FMAX = 3.0e38
L_LO, L_HI = 2.0 ** -60, 2.0 ** 60
RB = 512
BL = (128, 128, 256, 256, 256, 256, 256, 256, 256)
BO = tuple(sum(BL[:i]) for i in range(len(BL)))
LNC = 16
XD = (256, 256, 256, 256, 512, 512)
XO = tuple(sum(XD[:i]) for i in range(len(XD)))
PEEL, UNR = 4, 3
NACC = 8

NT = (((1,), (1,)), ((), ()))
TN = (((0,), (0,)), ((), ()))
f32, bf16, u32 = jnp.float32, jnp.bfloat16, jnp.uint32


def _pk(x):
    return pltpu.bitcast(x, u32)


def _upk(x):
    return pltpu.bitcast(x, bf16)


def _kernel(x_hbm, wqkv_hbm, wo_hbm, wr_hbm, wg_hbm, wu_hbm, wd_hbm, o_hbm,
            x_v, wqkv_v, wo_v, wr_v, wg_v, wu_v, wd_v,
            wk_p, wt_v, wo_p, xn_v, k_v, qm_v, vt_v, wrb_v, y_v, on_v, ot_v, out_v, b0_v, b4_v, p_s, l_s, z_s,
            sem_x, sem_w, sem_o):
    def xcopy(i):
        return pltpu.make_async_copy(x_hbm.at[pl.ds(XO[i], XD[i]), :], x_v.at[pl.ds(XO[i], XD[i]), :], sem_x.at[i])

    def wcopy(j):
        return pltpu.make_async_copy(wqkv_hbm.at[:, pl.ds(j * D, D)], wqkv_v.at[:, pl.ds(j * D, D)], sem_w.at[j])

    cp = {
        'wq': wcopy(0), 'wk': wcopy(1), 'wv': wcopy(2),
        'wr': pltpu.make_async_copy(wr_hbm, wr_v, sem_w.at[3]),
        'wo': pltpu.make_async_copy(wo_hbm, wo_v, sem_w.at[4]),
        'wg': pltpu.make_async_copy(wg_hbm, wg_v, sem_w.at[5]),
        'wu': pltpu.make_async_copy(wu_hbm, wu_v, sem_w.at[6]),
        'wd': pltpu.make_async_copy(wd_hbm, wd_v, sem_w.at[7]),
    }
    for i in range(len(XD)):
        cp[f'x{i}'] = xcopy(i)
    plan = {'start': ('x0', 'wr', 'wk', 'x1'), 'x0': ('x2',), 'x1': ('x3', 'x4'), 'x2': ('x5',),
            'x3': ('wq', 'wv'), 'x4': ('wg', 'wu'), 'x5': ('wd', 'wo')}

    def fire(point):
        for name in plan[point]:
            cp[name].start()

    x_waited = set()

    def need_rows(r1):
        for j in range(len(XD)):
            if XO[j] < r1 and j not in x_waited:
                x_waited.add(j)
                cp[f'x{j}'].wait()
                fire(f'x{j}')

    fire('start')

    ri = lax.broadcasted_iota(jnp.int32, (64, 128), 0)
    ci = lax.broadcasted_iota(jnp.int32, (64, 128), 1) & 63
    b0_v[...] = jnp.where(ri > ci, 0.0, NEG).astype(f32)
    b4_v[...] = jnp.where(ri <= ci, 0.0, NEG).astype(f32)
    for p in range(4):
        p_s[0, p, 160:192, :] = jnp.zeros((32, 128), u32)
        p_s[1, p, 0:32, :] = jnp.zeros((32, 128), u32)
    y_v[...] = jnp.zeros(y_v.shape, f32)
    lo = lax.broadcasted_iota(jnp.int32, (8, 128), 1) < 64

    def layer_norm(xb):
        mean = jnp.mean(xb, axis=-1, keepdims=True)
        xc = xb - mean
        var = jnp.mean(xc * xc, axis=-1, keepdims=True)
        return xc * lax.rsqrt(var + 1e-5)

    router = {}
    row16 = lax.broadcasted_iota(jnp.int32, (LNC, 1), 0)

    def ln_block(i):
        for c in range(BL[i] // LNC):
            r0 = BO[i] + c * LNC
            xnf = layer_norm(x_v[r0:r0 + LNC, :].astype(f32))
            xn_v[r0:r0 + LNC, :] = xnf.astype(bf16)
            rr = jnp.sum(xnf * wrb_v[0:1, :], axis=1, keepdims=True).astype(bf16).astype(f32)
            if 'best' not in router:
                router['best'], router['idx'] = rr, row16 + r0
            else:
                better = rr > router['best']
                router['best'] = jnp.where(better, rr, router['best'])
                router['idx'] = jnp.where(better, row16 + r0, router['idx'])

    def k_block(i):
        xn = xn_v[BO[i]:BO[i] + BL[i], :]
        kk = jnp.dot(xn, _upk(wk_p[...]), preferred_element_type=f32)
        k_v[pl.ds(BO[i] // 2, BL[i] // 2), :] = _pk(kk.astype(bf16))

    def qv_block(i):
        xn = xn_v[i * RB:(i + 1) * RB, :]
        qv = lax.dot_general(_upk(wt_v[...]), xn, NT, preferred_element_type=f32)
        for j in range(RB // 128):
            a = i * (RB // 128) + j
            cols = slice(j * 128, (j + 1) * 128)
            vt_v[a] = _pk(qv[D:2 * D, cols].astype(bf16))
            qp = _pk((qv[0:D, cols] * QSCALE).astype(bf16))
            for h in range(H):
                q = qp[8 * h:8 * h + 8]
                if h % 2 == 0:
                    qm_v[a, 0, 8 * h:8 * h + 8] = jnp.where(lo, q, 0)
                    qm_v[a, 1, 8 * h:8 * h + 8] = jnp.where(lo, 0, q)
                else:
                    r = pltpu.roll(q, 64, 1)
                    qm_v[a, 0, 8 * h:8 * h + 8] = jnp.where(lo, 0, r)
                    qm_v[a, 1, 8 * h:8 * h + 8] = jnp.where(lo, r, 0)

    nkb = len(BL)
    cp['wr'].wait()
    need_rows(BL[0])
    wr4 = wr_v[...].astype(f32).reshape(4, 128)
    wrb_v[...] = jnp.broadcast_to(jnp.concatenate([wr4[j:j + 1, :] for j in range(4)], axis=1), (8, D))
    ln_block(0)
    cp['wk'].wait()
    wk_p[...] = _pk(wqkv_v[:, D:2 * D])
    for i in range(nkb):
        if i + 1 < nkb:
            need_rows(BO[i + 1] + BL[i + 1])
        if i == nkb - 1:
            cp['wq'].wait()
            cp['wv'].wait()
        if i + 1 < nkb:
            ln_block(i + 1)
        k_block(i)
        if i == nkb - 1:
            wt_v[0:D // 2, :] = _pk(wqkv_v[:, 0:D].T)
            wt_v[D // 2:D, :] = _pk(wqkv_v[:, 2 * D:3 * D].T)

    rmax = jnp.max(router['best'])
    idx = jnp.min(jnp.where(router['best'] == rmax, router['idx'], S))
    idx = jnp.minimum(idx, S - 1)
    base = pl.multiple_of((idx // 16) * 16, 16)
    rsel = lax.broadcasted_iota(jnp.int32, (16, D), 0) == (idx - base)

    def ffn():
        xs = xn_v[pl.ds(base, 16), :].astype(f32)
        xb = jnp.broadcast_to(jnp.sum(jnp.where(rsel, xs, 0.0), axis=0, keepdims=True), (16, D))
        nc = F // 16
        accs = [None] * NACC
        for c in range(nc):
            f0 = 16 * c
            g = jnp.sum(wg_v[f0:f0 + 16, :].astype(f32) * xb, axis=1, keepdims=True)
            u = jnp.sum(wu_v[f0:f0 + 16, :].astype(f32) * xb, axis=1, keepdims=True)
            hh = (g * jax.nn.sigmoid(g) * u).astype(bf16).astype(f32)
            t = hh * wd_v[f0:f0 + 16, :].astype(f32)
            j = c * NACC // nc
            accs[j] = t if accs[j] is None else accs[j] + t
        acc = accs[0]
        for extra in accs[1:]:
            acc = acc + extra
        y = jnp.sum(acc, axis=0, keepdims=True) * jax.nn.sigmoid(jnp.full((1, D), rmax, f32))
        y_v[pl.ds(pl.multiple_of(base % QB, 16) + QB, 16), :] = jnp.where(rsel, y, 0.0)

    for i in range(S // RB):
        if i == 2:
            for name in ('wg', 'wu', 'wd'):
                cp[name].wait()
        qv_block(i)
        if i == 3:
            ffn()
    cp['wo'].wait()
    yblk = idx // QB
    wo_p[...] = _pk(wo_v[...])

    def ocopy(a):
        rows = pl.ds(pl.multiple_of(a * QB, QB), QB)
        return pltpu.make_async_copy(out_v.at[rows, :], o_hbm.at[rows, :], sem_o.at[0])

    def q_tile(a, e, g, p):
        r0 = (g * 128 + p * 32) // 2
        parts = []
        if p > 0:
            parts.append(jnp.zeros((32 * p, 128), bf16))
        parts.append(_upk(qm_v[a, e, r0:r0 + 16, :]))
        if p < 3:
            parts.append(jnp.zeros((32 * (3 - p), 128), bf16))
        return jnp.concatenate(parts, axis=0)

    chk = [jnp.ones((1, 128), f32), jnp.ones((1, 128), f32), jnp.zeros((8, 128), f32)]

    def stage_a(a, e, g, c0):
        if isinstance(a, int):
            kstart = (2 * a + e - 4 + c0) * 32
        else:
            kstart = pl.multiple_of((2 * a + e - 4) * 32, 32)
        kwin = _upk(k_v[pl.ds(kstart, 32 * (5 - c0)), g * 128:(g + 1) * 128])
        rhs = jnp.concatenate([q_tile(a, e, g, p) for p in range(4)], axis=1)
        st4 = jnp.dot(kwin, rhs, preferred_element_type=f32)
        for p in range(4):
            st = st4[:, p * 128:(p + 1) * 128]
            tot = None
            for c in range(c0, 5):
                sc = st[64 * (c - c0):64 * (c - c0) + 64]
                if c == 0:
                    sc = sc + b0_v[...]
                if c == 4:
                    sc = sc + b4_v[...]
                pc = jnp.exp2(sc)
                tot = pc if tot is None else tot + pc
                p_s[e, p, 32 * (c + e):32 * (c + e) + 32, :] = _pk(pc.astype(bf16))
            l = jnp.sum(tot, axis=0, keepdims=True)
            l_s[e, p] = jnp.broadcast_to(1.0 / l, (8, 128))
            chk[0] = jnp.minimum(chk[0], l)
            chk[1] = jnp.maximum(chk[1], l)

    def merge_halves(z0, z1):
        return jnp.where(lo, z0[0:8], z1[0:8]), pltpu.roll(jnp.where(lo, z1[8:16], z0[8:16]), 64, 1)

    def stage_b(a, e, g, slot, t0):
        slab = []
        for p in range(4):
            r0 = (g * 128 + p * 32) // 2
            ot = None
            for t in range(t0, 3):
                vt = _upk(vt_v[a - 2 + t, r0:r0 + 16, :])
                r = jnp.dot(vt, _upk(p_s[e, p, 64 * t:64 * (t + 1), :]), preferred_element_type=f32)
                ot = r if ot is None else ot + r
            on = ot * jnp.concatenate([l_s[e, p]] * 4, axis=0)
            fin = jnp.abs(on) <= FMAX
            chk[2] = jnp.where(fin[0:8] & fin[8:16] & fin[16:24] & fin[24:32], chk[2], 1.0)
            z = _pk(on.astype(bf16))
            if e == 0:
                z_s[p] = z
            else:
                slab += merge_halves(z_s[p], z)
        if e == 1:
            on_v[slot, :, g * 128:(g + 1) * 128] = _pk(_upk(jnp.concatenate(slab, axis=0)).T)

    def write_block(a, att):
        q0 = pl.multiple_of(a * QB, QB)
        yoff = pl.multiple_of(jnp.where(yblk == a, QB, 0), QB)
        res = att + (x_v[pl.ds(q0, QB), :].astype(f32) + xn_v[pl.ds(q0, QB), :].astype(f32)
                     + y_v[pl.ds(yoff, QB), :])
        out_v[pl.ds(q0, QB), :] = res.astype(bf16)

    def out_proj(a, slot):
        write_block(a, jnp.dot(_upk(on_v[slot]), _upk(wo_p[...]), preferred_element_type=f32))

    def c0_of(a, e):
        return max(0, 4 - (2 * a + e))

    def q_block(a, slot, first=False):
        static = isinstance(a, int)
        for gi in range(8):
            g, e = gi // 2, gi % 2
            stage_a(a, e, g, c0_of(a, e) if static else 0)
            if gi == 0:
                if not first:
                    stage_b(a - 1, 1, 3, (slot - 1) % UNR, max(0, 2 - (a - 1)) if static else 0)
            else:
                stage_b(a, (gi - 1) % 2, (gi - 1) // 2, slot, max(0, 2 - a) if static else 0)
        if not first:
            out_proj(a - 1, (slot - 1) % UNR)

    for a in range(PEEL):
        q_block(a, a % UNR, a == 0)
        if a >= 1:
            ocopy(a - 1).start()

    def main_loop(it, carry):
        chk[:] = carry
        a0 = PEEL + it * UNR
        for u in range(UNR):
            a = a0 + u
            q_block(a, (PEEL + u) % UNR)
            ocopy(a - 1).start()
        return tuple(chk)

    chk[:] = lax.fori_loop(0, (NQ - PEEL) // UNR, main_loop, tuple(chk))
    stage_b(NQ - 1, 1, 3, (NQ - 1) % UNR, 0)
    out_proj(NQ - 1, (NQ - 1) % UNR)
    ocopy(NQ - 1).start()
    for a in range(NQ):
        ocopy(a).wait()

    ok = (chk[0] >= L_LO) & (chk[1] <= L_HI)
    nbad = jnp.sum(jnp.where(ok, 0.0, 1.0)) + jnp.sum(chk[2])

    @pl.when(nbad != 0.0)
    def _():
        row = lax.broadcasted_iota(jnp.int32, (384, 128), 0)
        col = lax.broadcasted_iota(jnp.int32, (384, 128), 1) & 63

        def safe_block(a, carry):
            tiles = [jnp.maximum(a - 2 + t, 0) for t in range(3)]
            for g in range(4):
                kwin = jnp.concatenate(
                    [_upk(k_v[pl.ds(pl.multiple_of(tl * 64, 64), 64), g * 128:(g + 1) * 128]) for tl in tiles],
                    axis=0)
                zs = [None] * 4
                for e in range(2):
                    d = 256 + 64 * e + col - row
                    valid = (d >= 0) & (d < W) & (row + 128 * (a - 2) >= 0)
                    for p in range(4):
                        r0 = (g * 128 + p * 32) // 2
                        st = jnp.dot(kwin, q_tile(a, e, g, p), preferred_element_type=f32)
                        st = jnp.where(valid, st, NEG)
                        m = jnp.max(st, axis=0, keepdims=True)
                        pe = jnp.exp2(st - m)
                        linv = 1.0 / jnp.sum(pe, axis=0, keepdims=True)
                        vt = jnp.concatenate([_upk(vt_v[tl, r0:r0 + 16, :]) for tl in tiles], axis=1)
                        ot = jnp.dot(vt, pe.astype(bf16), preferred_element_type=f32)
                        z = _pk((ot * linv).astype(bf16))
                        if e == 0:
                            zs[p] = z
                        else:
                            ot_v[r0:r0 + 8, :], ot_v[r0 + 8:r0 + 16, :] = merge_halves(zs[p], z)
            write_block(a, lax.dot_general(_upk(ot_v[...]), _upk(wo_p[...]), TN, preferred_element_type=f32))
            ocopy(a).start()
            ocopy(a).wait()
            return carry

        lax.fori_loop(0, NQ, safe_block, 0)


@jax.jit
def pallas_parallel_sum__sliding_block__moe_arch_mod__prompt_kernel(
    A_x: jax.Array,
    A_wqkv: jax.Array,
    A_wo: jax.Array,
    B_x: jax.Array,
    B_w_r: jax.Array,
    B_w_gate: jax.Array,
    B_w_up: jax.Array,
    B_w_down: jax.Array,
):
    del B_x
    hbm = pl.BlockSpec(memory_space=pltpu.HBM)
    out = pl.pallas_call(
        _kernel,
        out_shape=jax.ShapeDtypeStruct((S, D), bf16),
        in_specs=[hbm] * 7,
        out_specs=hbm,
        scratch_shapes=[
            pltpu.VMEM((S, D), bf16),
            pltpu.VMEM((D, 3 * D), bf16),
            pltpu.VMEM((D, D), bf16),
            pltpu.VMEM((D,), bf16),
            pltpu.VMEM((F, D), bf16),
            pltpu.VMEM((F, D), bf16),
            pltpu.VMEM((F, D), bf16),
            pltpu.VMEM((D // 2, D), u32),
            pltpu.VMEM((D, D), u32),
            pltpu.VMEM((D // 2, D), u32),
            pltpu.VMEM((S, D), bf16),
            pltpu.VMEM((S // 2, D), u32),
            pltpu.VMEM((NQ, 2, D // 2, 128), u32),
            pltpu.VMEM((NQ, D // 2, 128), u32),
            pltpu.VMEM((8, D), f32),
            pltpu.VMEM((2 * QB, D), f32),
            pltpu.VMEM((UNR, QB // 2, D), u32),
            pltpu.VMEM((D // 2, 128), u32),
            pltpu.VMEM((S, D), bf16),
            pltpu.VMEM((64, 128), f32),
            pltpu.VMEM((64, 128), f32),
            pltpu.VMEM((2, 4, 192, 128), u32),
            pltpu.VMEM((2, 4, 8, 128), f32),
            pltpu.VMEM((4, 16, 128), u32),
            pltpu.SemaphoreType.DMA((len(XD),)),
            pltpu.SemaphoreType.DMA((8,)),
            pltpu.SemaphoreType.DMA((1,)),
        ],
        compiler_params=pltpu.CompilerParams(vmem_limit_bytes=80 * 2**20),
        name="fused_swa_mod",
    )(A_x.reshape(S, D), A_wqkv, A_wo, B_w_r, B_w_gate.T, B_w_up.T, B_w_down)
    return out.reshape(1, S, D)
```
